```python
import jax
import jax.numpy as jnp

def _softmax(x, axis=-1):
    return jax.nn.softmax(x, axis=axis)
def _gelu(x):
    return jax.nn.gelu(x, approximate=True)
def _silu(x):
    return jax.nn.silu(x)
def _sigmoid(x):
    return jax.nn.sigmoid(x)
def _layernorm(x, axis=-1, eps=1e-5):
    m = jnp.mean(x, axis=axis, keepdims=True)
    v = jnp.var(x, axis=axis, keepdims=True)
    return (x - m) / jnp.sqrt(v + eps)
def _scatter_add(tgt, idx, src, axis=0):
    return tgt.at[idx].add(src)
def _segment_sum(src, seg, n):
    return jax.ops.segment_sum(src, seg, n)
class _Rng:
    def __init__(self, key):
        self._k = key
    def _next(self):
        self._k, sub = jax.random.split(self._k)
        return sub
    def normal(self, shape):
        return jax.random.normal(self._next(), shape, dtype=jnp.bfloat16)
    def randint(self, lo, hi, shape):
        return jax.random.randint(self._next(), shape, lo, hi, dtype=jnp.int32)
    def uniform(self, shape, lo=0.0, hi=1.0):
        return jax.random.uniform(self._next(), shape, jnp.bfloat16, lo, hi)
    def permutation(self, n):
        return jax.random.permutation(self._next(), n)


kernel_name = 'standalone__mha_softmax__near_ridge'

def _fwd_setup_inputs():
    _rng = _Rng(jax.random.key(int.from_bytes(__import__("os").urandom(4), "little")))
    _w = (lambda a: (lambda t: t.astype(jnp.bfloat16) if jnp.issubdtype(t.dtype, jnp.floating) else t)(jnp.asarray(a)))
    B, H, Sq, Sk, D = 8, 16, 512, 1024, 256
    return {
        "q": _w((lambda *s: _rng.normal(s) * 0.05)(B, H, Sq, D)),
        "k": _w((lambda *s: _rng.normal(s) * 0.05)(B, H, Sk, D)),
        "v": _w((lambda *s: _rng.normal(s) * 0.05)(B, H, Sk, D)),
    }

def _fwd_reference(q, k, v):
    scale = q.shape[-1] ** -0.5
    scores = jnp.einsum("bhqd,bhkd->bhqk", q, k) * scale
    p = _softmax(scores, axis=-1)
    return jnp.einsum("bhqk,bhkd->bhqd", p, v)


def setup_inputs():
    _inp = _fwd_setup_inputs()
    _gk = jax.random.fold_in(jax.random.key(int.from_bytes(__import__("os").urandom(4), "little")), 2**31 - 1)
    _shapes = [[8, 16, 512, 256]]
    _dtypes = ['bfloat16']
    _gks = jax.random.split(_gk, len(_shapes))
    _gs = [jax.random.normal(k, s, dtype=jnp.dtype(d)) * 0.05 for k, s, d in zip(_gks, _shapes, _dtypes)]
    _inp["grad_out"] = _gs[0]
    return _inp

def reference(q, k, v, grad_out):
    _const = dict()
    def _f(*_d):
        return _fwd_reference(**{'q': _d[0], 'k': _d[1], 'v': _d[2], **_const})
    _out, _vjp = jax.vjp(_f, q, k, v)
    _grads = _vjp(grad_out)
    _out0 = jnp.asarray(_out)
    return (_out0, *[jnp.asarray(_g) for _g in _grads])
```

```python
import functools, math
import jax, jax.numpy as jnp
from jax import lax
from jax.experimental import pallas as pl
from jax.experimental.pallas import tpu as pltpu

NT = (((1,), (1,)), ((), ()))
NN = (((1,), (0,)), ((), ()))
f32 = jnp.float32; bf16 = jnp.bfloat16; u32 = jnp.uint32
D = 256; Sq = 512; Sk = 1024
GK = 16; GQ = 128
HL = "abcdefgh"

def dot(a, b, dn=NN):
    return lax.dot_general(a, b, dn, preferred_element_type=f32)

def dot2(a, b, dn=NN):
    h = a.shape[0] // 2
    return jnp.concatenate([dot(a[:h], b, dn), dot(a[h:], b, dn)], axis=0)

def split_rows(x, g):
    r, c = x.shape
    y = x.reshape(r // (2 * g), 2, g, c)
    return y[:, 0].reshape(r // 2, c), y[:, 1].reshape(r // 2, c)

def merge_rows(a, b, g):
    r, c = a.shape
    return jnp.stack([a.reshape(r // g, g, c), b.reshape(r // g, g, c)], axis=1).reshape(2 * r, c)

def split_cols(x):
    n = x.shape[1] // 128
    ev = [x[:, 128 * i:128 * (i + 1)] for i in range(0, n, 2)]
    od = [x[:, 128 * i:128 * (i + 1)] for i in range(1, n, 2)]
    cat = lambda l: l[0] if len(l) == 1 else jnp.concatenate(l, axis=1)
    return cat(ev), cat(od)

def merge_cols(a, b):
    parts = []
    for i in range(a.shape[1] // 128):
        parts += [a[:, 128 * i:128 * (i + 1)], b[:, 128 * i:128 * (i + 1)]]
    return jnp.concatenate(parts, axis=1)

def blocks(x, g):
    t, b = split_rows(x, g)
    return (*split_cols(t), *split_cols(b))

pk = lambda x: pltpu.bitcast(x, u32)
upk = lambda x: pltpu.bitcast(x, bf16)
cat1 = lambda *xs: jnp.concatenate(xs, axis=1)
cat0 = lambda *xs: jnp.concatenate(xs, axis=0)

def red0(x, op, nacc):
    R, C = x.shape
    y = op(x.reshape(R // (8 * nacc), 8 * nacc, C), axis=0)
    return op(y, axis=0, keepdims=True)

DEF = dict(
    order="Sa Sb Pa Oa Pb Va Ob Ka Qa Vb Qb Kb",
    dl2=1, dl3=1, dlz=2, fly=8, dl_out_t=3, dl_out=2, dl_delta=2, dl_bb=0,
    g1=2, g2=4, g3=1, capv=2.5, caps=0.7, verbose=False, gs=1, sspan=1.0, pw=4, look=30, p1frac=None, ebase=1.0,
)
SUB = 512

def make_plan(C):
    groups = C["order"].split()
    names = []
    for g in groups:
        names += [f"{g}{n}" for n in range(4 if g[0] == "S" else 7)]
    idx = {n: i for i, n in enumerate(names)}
    N = len(names)
    dur = [512 if n[0] == "S" else 256 for n in names]
    V = [0.0] * N; S = [0.0] * N
    own = dict(S=(620, 128), O=(165, 32), Q=(165, 32), V=(140, 64), K=(140, 64), P=(60, 128))
    for i, n in enumerate(names):
        v, s = own[n[0]]
        k = int(n[2:])
        if n[0] in "OQVK" and k >= 5:
            s = 0
        V[i] += v; S[i] += s
        if n[0] in "VK" and k >= 5:
            V[i] += (320 if n[0] == "V" else 450) * C["ebase"]; S[i] += 64
        if n[0] in "OQ" and k >= 5:
            V[i] += 170 * C["ebase"]
        if n[0] in "OQ" and k == 6:
            for d_, (v2, s2) in enumerate([(350, 16), (250, 48)] if n[0] == "O" else [(150, 16), (150, 48)]):
                if i + 1 + d_ < N:
                    V[i + 1 + d_] += v2 * C["ebase"]; S[i + 1 + d_] += s2
    first = lambda g: idx[g + "0"]
    last = lambda g: idx[g + ("3" if g[0] == "S" else "6")]
    off = lambda i: 1 if names[i][0] == "S" else 2
    pw = C["pw"]
    phi = lambda i, v=0, s=0: dur[i] * (((V[i] + v) / dur[i] / C["capv"]) ** pw + ((S[i] + s) / dur[i] / C["caps"]) ** pw)
    def fill(lo, hi, n, v, s, maxper=None):
        cnt = {}
        for _ in range(n):
            cand = [i for i in range(lo, hi + 1) if maxper is None or cnt.get(i, 0) < maxper * dur[i] // 256]
            b = min(cand, key=lambda i: phi(i, v, s) - phi(i))
            cnt[b] = cnt.get(b, 0) + 1
            V[b] += v; S[b] += s
        return sorted(cnt.items())
    def unfill(items, v, s):
        for i, c_ in items:
            V[i] -= c_ * v; S[i] -= c_ * s
    def latest(consumer, dl):
        g = consumer - 1
        while g + off(g) + dl > consumer:
            g -= 1
        return g
    heads = sorted({g[1] for g in groups})
    plan = {}
    P1 = (50 + C["g1"], 0); P2 = (27 + C["g2"], 9); DS = (57 + C["g3"], 7)
    COST = dict(y=(340, 96), z=(300, 56), w=(54, 10), u=(54, 10), t=(60, 0))
    total = lambda: sum(phi(i) for i in range(N))
    def place(kind, h):
        if kind in COST:
            key = kind + h
            if key in plan:
                unfill(plan[key], *COST[kind])
            if kind == "t":
                plan[key] = fill(first("O" + h), first("O" + h) + 3, 1, *COST[kind])
                return
            cons = dict(y=min(first("P" + h), first("O" + h)), z=first("Q" + h), w=min(first("P" + h), first("V" + h)), u=first("K" + h))[kind]
            plan[key] = fill(max(0, cons - C["look"]), cons - 1 - C["dlz"], 4 if kind in "yz" else 8, *COST[kind], maxper=1 if kind in "yz" else None)
        elif kind == "sm":
            for key, cst in (("p1" + h + "1", P1), ("p1" + h + "0", P1), ("p2" + h, P2)):
                if key in plan:
                    unfill(plan[key], *cst)
            end = latest(min(first("O" + h), first("V" + h)), 0)
            s3 = last("S" + h)
            best = None
            for split in range(s3 + 1, end):
                st2 = max(split + off(split) + C["dl_bb"] - 1, split + 1)
                if st2 > end:
                    continue
                a_ = fill(s3 + 1, split, 16, *P1); b_ = fill(s3 - 1, split, 16, *P1); c_ = fill(st2, end, 64, *P2)
                m = total()
                unfill(a_, *P1); unfill(b_, *P1); unfill(c_, *P2)
                if best is None or m < best[0]:
                    best = (m, split, st2)
            _, split, st2 = best
            plan["p1" + h + "1"] = fill(s3 + 1, split, 16, *P1)
            plan["p1" + h + "0"] = fill(s3 - 1, split, 16, *P1)
            plan["p2" + h] = fill(st2, end, 64, *P2)
        else:
            key = "ds" + h
            if key in plan:
                unfill(plan[key], *DS)
            lo = max(last("O" + h) + 1 + C["dl_delta"], last("P" + h) + 1)
            plan[key] = fill(lo, latest(min(first("K" + h), first("Q" + h)), 0), 64, *DS)
    for rnd in range(4):
        for h in heads:
            for kind in ("y", "w", "t", "z", "u"):
                place(kind, h)
        for h in heads:
            place("sm", h); place("ds", h)
    if C["verbose"]:
        for k, v in plan.items():
            print(k, " ".join(f"{names[i]}:{c}" for i, c in v))
        print(" ".join(f"{names[i]}:{V[i]/dur[i]:.1f}/{S[i]/dur[i]:.2f}" for i in range(N)))
    return groups, names, idx, plan, heads


def build(nobc=True, **kw):
    C = dict(DEF); C.update(kw)
    scale = D ** -0.5
    c = scale * math.log2(math.e)
    groups, names, sidx, PLAN, heads = make_plan(C)
    hb = len(heads)
    NPER = 10

    def kernel(q_ref, k_ref, v_ref, do_ref, o_ref, dq_ref, dk_ref, dv_ref, *scr):
        per = [dict(zip(("s", "p", "ds", "kt", "vt", "mp", "vn", "vn5", "w", "w5"), scr[NPER * h:NPER * (h + 1)])) for h in range(hb)]
        mo = list(scr[NPER * hb:NPER * hb + 2]); mv = list(scr[NPER * hb + 2:NPER * hb + 4])
        def nxt(l):
            l.reverse()
            return l[0]
        i = pl.program_id(0)
        z0 = lax.shift_right_logical(i, 20)
        z1 = lax.shift_right_logical(i, 21)
        z2 = lax.shift_right_logical(i, 22)
        never = lax.broadcasted_iota(jnp.int32, (8, 128), 0) < z0
        st = [dict() for _ in range(hb)]
        delayed = []; res = {}; todo = {}

        def nv(n):
            return never if n == 1 else jnp.concatenate([never] * n, axis=1)

        def token(tok, delay):
            delayed.append([tok, delay])

        def deadline(x, delay):
            for t in range(x.shape[1] // 128):
                token(pk(jnp.broadcast_to(x[:, 128 * t:128 * (t + 1)], (8, 128))), delay)

        def tie(x):
            now = [e[0] for e in delayed if e[1] <= 0]
            delayed[:] = [[e[0], e[1] - 1] for e in delayed if e[1] > 0]
            if not now:
                return x
            head = jnp.where(never, functools.reduce(lambda a, b: a | b, now), pk(x[0:16, 0:128]))
            top = upk(head) if x.shape[1] == 128 else cat1(upk(head), x[0:16, 128:])
            return cat0(top, x[16:])

        def gate(x, trig, n=None):
            w = x.shape[1] // 128
            n = w if n is None else min(n, w)
            if trig is None:
                return x
            if trig.dtype != x.dtype:
                trig = pltpu.bitcast(trig, x.dtype)
            g = jnp.where(nv(n), trig if n == 1 else jnp.concatenate([trig] * n, axis=1), x[:, :128 * n])
            return g if n == w else cat1(g, x[:, 128 * n:])

        def trig_of(name, frac):
            m = res[name]
            if name[0] in "OQ":
                k = min(int(frac * 32), 31)
                return m[8 * (k % 16):8 * (k % 16) + 8, 128 * (k // 16):128 * (k // 16) + 128]
            rows = m.shape[0] // 2 if name[0] in "VKP" else m.shape[0]
            k = min(int(frac * (rows // 8)), rows // 8 - 1)
            return m[8 * k:8 * k + 8, 0:128]

        def slot(name, lhs, rhs, d):
            for f in todo.pop(sidx[name], []):
                f()
            m = d(lhs(), tie(rhs()))
            res[name] = m
            return m

        def plan(key, chunk_fn, after_group=None, final=None, off=None):
            items = PLAN[key]
            base = 0
            for n, (si, cnt) in enumerate(items):
                name = names[si]
                def run(name=name, cnt=cnt, base=base, last=(n == len(items) - 1)):
                    for k in range(cnt):
                        chunk_fn(base + k, lambda x=0.0, k=k: trig_of(name, (k + x) / cnt))
                    if after_group is not None:
                        after_group(last)
                    if last and final is not None:
                        final()
                todo.setdefault(si + (off if off is not None else (1 if name[0] == "S" else 2)), []).append(run)
                base += cnt

        def strassen(g, A, B, scr_, d):
            ms = []
            for n, (ja, jb) in enumerate([(2, 2), (1, 5), (4, 1), (3, 0), (0, 6), (6, 3), (5, 4)]):
                m = slot(f"{g}{n}", lambda: A(ja), lambda: B(jb), d)
                ms.append(m)
                if n < 5:
                    scr_[z0, n] = m
            L = lambda n: scr_[z2, n]
            return (L(0) + L(1) - L(2) + ms[5], L(4) + L(2), L(3) + L(1), L(0) - L(3) + L(4) + ms[6])

        def gate_rows(x, trig, rows):
            hd = pk(x[0:rows])
            hd = cat0(*[gate(hd[8 * r:8 * r + 8], trig) for r in range(rows // 16)])
            return cat0(upk(hd), x[rows:])

        def gate8(x, trig, n):
            return cat0(*[gate(x[8 * r:8 * r + 8], trig) if r < n else x[8 * r:8 * r + 8] for r in range(x.shape[0] // 8)])

        def set_chunk(h, name, ch, tf):
            ref, sc = (v_ref, per[h]["vt"]) if name == "VT" else (k_ref, per[h]["kt"])
            us = [[] for _ in range(5)]
            for g in range(8):
                r0 = 256 * ch + 32 * g
                x = ref[h, r0:r0 + 32].astype(f32)
                tr = tf(g / 8 * C["sspan"])
                a = gate8(x[:16, :128], tr, C["gs"]); b = x[:16, 128:]; cc = x[16:, :128]; d = gate8(x[16:, 128:], tr, C["gs"])
                for l, u in zip(us, [a + d, b + d, a + cc, b - a, cc - d]):
                    l.append(u)
                if name == "VT":
                    rs = slice(128 * ch + 16 * g, 128 * ch + 16 * (g + 1))
                    wz = (z0, z1)[g % 2]
                    per[h]["vn"][wz, 0, rs, :] = cat1(us[0][-1], us[1][-1]).astype(bf16)
                    per[h]["vn"][wz, 1, rs, :] = cat1(us[2][-1], us[3][-1]).astype(bf16)
                    if g % 2 == 1:
                        r5 = 64 * ch + 16 * (g // 2)
                        per[h]["vn5"][z0, r5:r5 + 16, :] = cat1(us[4][-2], us[4][-1]).astype(bf16)
            x11, _, _, x22 = blocks(ref[h, 256 * ch:256 * (ch + 1)], GK)
            for j, y in enumerate([x11, x22] + [cat0(*l).astype(bf16) for l in us]):
                sc[z0, j, :, 128 * ch:128 * (ch + 1)] = pk(y.T)

        def set_token(h, name):
            sc = per[h]["vt"] if name == "VT" else per[h]["kt"]
            token(sc[z2, 0, 0:8, 0:128], C["dlz"])
            if name == "VT":
                token(pk(per[h]["vn"][z2, 0, 0:16, 0:128]) | pk(per[h]["vn5"][z2, 0:16, 0:128]), C["dlz"])

        def w_chunk(h, which, g, tf):
            ref = (do_ref, q_ref)[which]
            r0 = 256 * (g // 4) + 32 * (g % 4)
            t5 = []
            for e in range(2):
                tr = tf(e / 2)
                x = ref[h, r0 + 16 * e:r0 + 16 * e + 16].astype(f32); y = ref[h, r0 + 128 + 16 * e:r0 + 144 + 16 * e].astype(f32)
                a = gate8(x[:, :128], tr, C["gs"]); b = x[:, 128:]; cc = y[:, :128]; d = gate8(y[:, 128:], tr, C["gs"])
                rs = slice(32 * g + 16 * e, 32 * g + 16 * e + 16)
                wz = (z0, z1)[e]
                per[h]["w"][wz, which, 0, rs, :] = cat1(a + d, cc + d).astype(bf16)
                per[h]["w"][wz, which, 1, rs, :] = cat1(a + b, cc - a).astype(bf16)
                t5.append(b - d)
            per[h]["w5"][z0, which, 16 * g:16 * (g + 1), :] = cat1(*t5).astype(bf16)

        def w_token(h, which):
            token(pk(per[h]["w"][z2, which, 0, 0:16, 0:128]) | pk(per[h]["w5"][z2, which, 0:16, 0:128]), C["dlz"])

        def getW(h, which):
            ref = (do_ref, q_ref)[which]
            def f(j):
                if j == 0:
                    return cat0(ref[h, 0:128, 0:128], ref[h, 256:384, 0:128])
                if j == 1:
                    return cat0(ref[h, 128:256, 128:256], ref[h, 384:512, 128:256])
                if j < 6:
                    return per[h]["w"][z2, which, (j - 2) // 2, :, 128 * (j % 2):128 * (j % 2 + 1)]
                return merge_rows(per[h]["w5"][z0, which, :, 0:128], per[h]["w5"][z0, which, :, 128:256], 16)
            return f

        def S(h):
            fly = C["fly"]; R = 8 * fly
            st[h]["m"] = []
            for t in range(2):
                acc = None
                for u in range(2):
                    s = slot(f"S{HL[h]}{2 * t + u}", lambda: k_ref[h, SUB * u:SUB * (u + 1)], lambda: q_ref[h, 256 * t:256 * (t + 1)], lambda a, b: dot(a, b, NT) * c)
                    for g in range(SUB // R):
                        x = s[R * g:R * (g + 1)]
                        mx = jnp.max(x.reshape(fly, 8, 256), axis=0)
                        acc = mx if acc is None else jnp.maximum(acc, mx)
                        x = cat0(x[:R - 8], jnp.where(nv(2), acc, x[R - 8:]))
                        per[h]["s"][z0, SUB * u + R * g:SUB * u + R * (g + 1), 256 * t:256 * (t + 1)] = x
                m = jnp.max(acc, axis=0, keepdims=True)
                st[h]["m"].append(m)
                st[h][f"m8{t}"] = jnp.broadcast_to(m, (8, 256))
                deadline(m, 1)

        def p1_chunk(h, t, g, trig):
            mg = gate(st[h][f"m8{t}"], trig(), C["g1"])
            e = jnp.exp2(per[h]["s"][z0, 64 * g:64 * (g + 1), 256 * t:256 * (t + 1)].reshape(8, 8, 256) - mg[None])
            e = e.reshape(2, 32, 256)
            e = e[0] + e[1]
            st[h][f"acc{t}"] = e if g == 0 else st[h][f"acc{t}"] + e

        def p1_final(h, t):
            l = jnp.sum(st[h][f"acc{t}"], axis=0, keepdims=True)
            st[h][f"bb{t}"] = st[h]["m"][t] + jnp.log2(l)
            if "bb0" in st[h] and "bb1" in st[h]:
                bb = cat1(st[h]["bb0"], st[h]["bb1"])
                comb = bb[:, 0:128] + bb[:, 128:256] + bb[:, 256:384] + bb[:, 384:512]
                bb = jnp.where(nv(4)[0:1], jnp.concatenate([comb] * 4, axis=1), bb)
                st[h]["b8"] = jnp.broadcast_to(bb, (8, 512))
                deadline(bb, C["dl_bb"] + st[h].get("bbx", 0))

        def p2_chunk(h, g, tr):
            bg = gate(st[h]["b8"], tr(), C["g2"])
            r0 = 32 * (g // 2) + 8 * (g % 2)
            a, b = split_cols(jnp.exp2(per[h]["s"][z0, r0:r0 + 8, :] - bg))
            cc, d = split_cols(jnp.exp2(per[h]["s"][z0, r0 + 16:r0 + 24, :] - bg))
            wz = (z0, z1)[g % 2]
            for j, x in enumerate([a, d, a + d, cc + d, a + b, cc - a, b - d, b, cc]):
                per[h]["p"][wz, j, 8 * g:8 * (g + 1), :] = x.astype(bf16)

        getP = lambda h: (lambda j: per[h]["p"][z2, j])
        getDS = lambda h: (lambda j: per[h]["ds"][z2, j])
        getT = lambda h, name: (lambda j: upk(per[h][name][z0, j]))

        def t_chunk(h, k, trig):
            st[h]["doT"] = gate_rows(do_ref[h], trig(), 16).T

        def O(h):
            c11, c12, c21, c22 = strassen("O" + HL[h], getT(h, "vt"), getP(h), nxt(mo), dot)
            top = merge_cols(c11, c12); bot = merge_cols(c21, c22)
            o_ref[h] = cat1(top.T, bot.T).astype(bf16)
            token(pk(o_ref[z2 + h, 0:16, 0:128]), C["dl_out_t"])
            dot_ = st[h]["doT"].astype(f32)
            delta = red0(dot_[:128] * top + dot_[128:] * bot, jnp.sum, 2)
            deadline(delta, C["dl_delta"])
            st[h]["d8"] = jnp.broadcast_to(cat1(*split_cols(delta)), (8, 512))

        def V(h):
            c11, c12, c21, c22 = strassen("V" + HL[h], getP(h), getW(h, 0), nxt(mv), dot2)
            dv_ref[h] = merge_rows(cat1(c11, c12), cat1(c21, c22), GK).astype(bf16)
            token(pk(dv_ref[z2 + h, 0:16, 0:128]), C["dl_out"])

        def getVN(h, j):
            if j < 2:
                t, bt = split_rows(v_ref[h], GK)
                return t[:, 0:128] if j == 0 else bt[:, 128:256]
            if j < 6:
                return per[h]["vn"][z2, (j - 2) // 2, :, 128 * (j % 2):128 * (j % 2 + 1)]
            return merge_rows(per[h]["vn5"][z0, :, 0:128], per[h]["vn5"][z0, :, 128:256], 16)

        def P_(h):
            W = getW(h, 0)
            for n, (ja, jb) in enumerate([(2, 2), (1, 4), (5, 1), (3, 6), (6, 0), (0, 3), (4, 5)]):
                per[h]["mp"][z0, n] = slot(f"P{HL[h]}{n}", lambda: getVN(h, ja), lambda: W(jb), lambda a, b: dot2(a, b, NT))

        def ds_chunk(h, g, tr):
            d8 = gate(st[h]["d8"], tr(), C["g3"])
            de, do_ = d8[:, 0:256], d8[:, 256:512]
            rs = slice(8 * g, 8 * (g + 1))
            M = lambda n: per[h]["mp"][z2, n, rs, :]
            m1 = M(0); n4 = M(1); n5 = M(2); n2 = M(4); n3 = M(5)
            c21 = n2 + (n4 - de)
            c12 = (n3 - do_) + n5
            c11 = (m1 + M(3)) - (n4 + de) + n5
            c22 = (m1 + M(6)) - (n3 + do_) + n2
            pp = lambda j: per[h]["p"][z2, j, rs, :].astype(f32)
            a = c11 * pp(0); b = c12 * pp(7); cc = c21 * pp(8); d = c22 * pp(1)
            wz = (z0, z1)[g % 2]
            for j, x in enumerate([a, d, a + d, cc + d, a + b, cc - a, b - d]):
                per[h]["ds"][wz, j, rs, :] = x.astype(bf16)

        def K(h):
            c11, c12, c21, c22 = strassen("K" + HL[h], getDS(h), getW(h, 1), nxt(mv), dot2)
            dk_ref[h] = (merge_rows(cat1(c11, c12), cat1(c21, c22), GK) * scale).astype(bf16)
            token(pk(dk_ref[z2 + h, 0:16, 0:128]), C["dl_out"])

        def Q_(h):
            c11, c12, c21, c22 = strassen("Q" + HL[h], getT(h, "kt"), getDS(h), nxt(mo), dot)
            top = merge_cols(c11, c12) * scale; bot = merge_cols(c21, c22) * scale
            dq_ref[h] = cat1(top.T, bot.T).astype(bf16)
            token(pk(dq_ref[z2 + h, 0:16, 0:128]), C["dl_out_t"])

        P = functools.partial
        for h in range(hb):
            x = HL[h]
            if names[PLAN["p1" + x + "1"][-1][0]][0] == "S":
                st[h]["bbx"] = 1
            plan("y" + x, P(set_chunk, h, "VT"), after_group=lambda last, h=h: set_token(h, "VT"), off=1)
            plan("z" + x, P(set_chunk, h, "KT"), after_group=lambda last, h=h: set_token(h, "KT"), off=1)
            plan("w" + x, P(w_chunk, h, 0), after_group=lambda last, h=h: w_token(h, 0), off=1)
            plan("u" + x, P(w_chunk, h, 1), after_group=lambda last, h=h: w_token(h, 1), off=1)
            plan("t" + x, P(t_chunk, h), off=1)
            plan("p1" + x + "0", P(p1_chunk, h, 0), final=P(p1_final, h, 0))
            plan("p1" + x + "1", P(p1_chunk, h, 1), final=P(p1_final, h, 1))
            plan("p2" + x, P(p2_chunk, h), after_group=lambda last, h=h: token(pk(per[h]["p"][z2, 0, 0:16, 0:128]), C["dl2"]))
            plan("ds" + x, P(ds_chunk, h), after_group=lambda last, h=h: token(pk(per[h]["ds"][z2, 0, 0:16, 0:128]), C["dl3"]))
        fns = dict(S=S, O=O, V=V, P=P_, K=K, Q=Q_)
        for tok in groups:
            fns[tok[0]](HL.index(tok[1]))
        assert not todo, todo

    def fn(q, k, v, do):
        B, H = q.shape[:2]
        BH = B * H
        q3, k3, v3, do3 = (x.reshape(BH, x.shape[2], D) for x in (q, k, v, do))
        qspec = pl.BlockSpec((hb, Sq, D), lambda i: (i, 0, 0))
        kspec = pl.BlockSpec((hb, Sk, D), lambda i: (i, 0, 0))
        V_ = pltpu.VMEM
        per = [V_((1, Sk, Sq), f32), V_((1, 9, 512, 256), bf16), V_((1, 7, 512, 256), bf16),
               V_((1, 7, 64, 512), u32), V_((1, 7, 64, 512), u32), V_((1, 7, 512, 256), f32),
               V_((1, 2, 512, 256), bf16), V_((1, 256, 256), bf16), V_((1, 2, 2, 256, 256), bf16), V_((1, 2, 128, 256), bf16)]
        outs = pl.pallas_call(
            kernel,
            grid=(BH // hb,),
            in_specs=[qspec, kspec, kspec, qspec],
            out_specs=[qspec, qspec, kspec, kspec],
            out_shape=[jax.ShapeDtypeStruct(q3.shape, bf16), jax.ShapeDtypeStruct(q3.shape, bf16),
                       jax.ShapeDtypeStruct(k3.shape, bf16), jax.ShapeDtypeStruct(k3.shape, bf16)],
            scratch_shapes=per * hb + [V_((1, 5, 128, 256), f32), V_((1, 5, 128, 256), f32), V_((1, 5, 512, 128), f32), V_((1, 5, 512, 128), f32)],
            compiler_params=pltpu.CompilerParams(dimension_semantics=("arbitrary",), vmem_limit_bytes=110 * 1024 * 1024, disable_bounds_checks=nobc),
        )(q3, k3, v3, do3)
        o, dq, dk, dv = outs
        return o.reshape(q.shape), dq.reshape(q.shape), dk.reshape(k.shape), dv.reshape(k.shape)
    return fn


_FN = build()


@jax.jit
def pallas_standalone__mha_softmax__near_ridge_kernel(q, k, v, grad_out):
    return _FN(q, k, v, grad_out)
```

```python
import functools
import math

import jax
import jax.numpy as jnp
from jax import lax
from jax.experimental import pallas as pl
from jax.experimental.pallas import tpu as pltpu

f32 = jnp.float32
bf16 = jnp.bfloat16
u32 = jnp.uint32
NT = (((1,), (1,)), ((), ()))
NN = (((1,), (0,)), ((), ()))

D = 256
SQ = 512
SK = 1024
HB = 2
GK = 16
SUB = 512
FLY = 16
R1 = 32

ORDER = ['Sa', 'Sb', 'Pa', 'Va', 'Pb', 'Oa', 'Qa', 'Ob', 'Ka', 'Vb', 'Qb', 'Kb']
SLOTS = [f"{g}{n}" for g in ORDER for n in range(4 if g[0] == "S" else 7)]
SLOT_INDEX = {n: i for i, n in enumerate(SLOTS)}

PLAN_LOOP = {
    'ya': [('Sa0', 2), ('Sa1', 2)],
    'wa': [('Sa2', 3), ('Sa3', 3), ('Sb0', 1), ('Sb1', 1)],
    'za': [('Pa5', 1), ('Pa6', 1), ('Va0', 1), ('Pb2', 1)],
    'ua': [('Ob0', 1), ('Ob2', 3), ('Ob3', 3), ('Ob4', 1)],
    'yb': [('Sb0', 1), ('Va1', 1), ('Va2', 1), ('Va4', 1)],
    'wb': [('Sb2', 1), ('Pa1', 1), ('Pa5', 3), ('Pa6', 3)],
    'zb': [('Ka2', 1), ('Ka3', 1), ('Ka4', 1), ('Vb0', 1)],
    'ub': [('Qb0', 2), ('Qb1', 2), ('Qb2', 2), ('Qb3', 1), ('Qb4', 1)],
    'p1a1': [('Sb0', 2), ('Sb1', 15), ('Sb2', 15)],
    'p1a0': [('Sa2', 13), ('Sa3', 13), ('Sb0', 2), ('Sb1', 2), ('Sb2', 2)],
    'p2a': [('Sb3', 18), ('Pa0', 10), ('Pa1', 8), ('Pa2', 10), ('Pa3', 9), ('Pa4', 9)],
    'd1a': [('Va0', 7), ('Va1', 5), ('Va2', 5), ('Va3', 14), ('Va4', 5), ('Pb0', 14), ('Pb1', 14)],
    'dsa': [('Pb3', 16), ('Pb4', 16), ('Pb5', 16), ('Pb6', 2), ('Oa0', 3), ('Oa1', 4), ('Oa2', 4), ('Oa3', 2), ('Oa4', 1)],
    'p1b1': [('Oa0', 8), ('Oa1', 7), ('Oa2', 7), ('Oa3', 10)],
    'p1b0': [('Pb6', 30), ('Oa0', 1), ('Oa3', 1)],
    'p2b': [('Oa4', 11), ('Qa0', 9), ('Qa1', 8), ('Qa2', 12), ('Qa3', 12), ('Qa4', 12)],
    'd1b': [('Ob0', 3), ('Ob1', 4), ('Ob2', 4), ('Ob3', 4), ('Ob4', 7), ('Ka0', 11), ('Ka1', 10), ('Ka2', 7), ('Ka3', 7), ('Ka4', 7)],
    'dsb': [('Vb0', 7), ('Vb1', 15), ('Vb2', 14), ('Vb3', 14), ('Vb4', 14)],
}
PLAN_FIRST = {
    'ya': [('Sa2', 1), ('Sa3', 1), ('Sb0', 1), ('Sb1', 1)],
    'wa': [('Sa2', 2), ('Sa3', 2), ('Sb0', 2), ('Sb1', 2)],
    'za': [('Pa5', 1), ('Pa6', 1), ('Va0', 1), ('Pb2', 1)],
    'ua': [('Ob0', 1), ('Ob2', 3), ('Ob3', 3), ('Ob4', 1)],
    'yb': [('Va1', 1), ('Va2', 1), ('Va3', 1), ('Va4', 1)],
    'wb': [('Pa0', 4), ('Pa5', 2), ('Pa6', 2)],
    'zb': [('Ka2', 1), ('Ka3', 1), ('Ka4', 1), ('Vb0', 1)],
    'ub': [('Qb0', 2), ('Qb1', 2), ('Qb2', 2), ('Qb3', 1), ('Qb4', 1)],
    'p1a1': [('Sb0', 5), ('Sb1', 5), ('Sb2', 22)],
    'p1a0': [('Sa2', 10), ('Sa3', 10), ('Sb0', 4), ('Sb1', 4), ('Sb2', 4)],
    'p2a': [('Sb3', 19), ('Pa0', 5), ('Pa1', 10), ('Pa2', 10), ('Pa3', 10), ('Pa4', 10)],
    'd1a': [('Va0', 8), ('Va1', 6), ('Va2', 6), ('Va3', 6), ('Va4', 6), ('Pb0', 16), ('Pb1', 16)],
    'dsa': [('Pb3', 16), ('Pb4', 16), ('Pb5', 16), ('Pb6', 2), ('Oa0', 3), ('Oa1', 4), ('Oa2', 4), ('Oa3', 2), ('Oa4', 1)],
    'p1b1': [('Oa0', 8), ('Oa1', 7), ('Oa2', 7), ('Oa3', 10)],
    'p1b0': [('Pb6', 30), ('Oa0', 1), ('Oa3', 1)],
    'p2b': [('Oa4', 11), ('Qa0', 9), ('Qa1', 8), ('Qa2', 12), ('Qa3', 12), ('Qa4', 12)],
    'd1b': [('Ob0', 3), ('Ob1', 4), ('Ob2', 4), ('Ob3', 4), ('Ob4', 7), ('Ka0', 11), ('Ka1', 10), ('Ka2', 7), ('Ka3', 7), ('Ka4', 7)],
    'dsb': [('Vb0', 7), ('Vb1', 15), ('Vb2', 14), ('Vb3', 14), ('Vb4', 14)],
}

INS = ("q", "k", "v", "do")
ROWS = dict(q=SQ, do=SQ, k=SK, v=SK, o=SQ, dq=SQ, dk=SK, dv=SK)
OFF = dict(q=0, do=HB * SQ, k=2 * HB * SQ, v=2 * HB * SQ + HB * SK,
           o=0, dq=HB * SQ, dk=2 * HB * SQ, dv=2 * HB * SQ + HB * SK)
TOT = 2 * HB * (SQ + SK)
PER_HEAD = ("s", "p", "ds", "kt", "vt", "mp", "vn", "vn5", "w", "w5")


def dot(a, b, dn=NN):
    return lax.dot_general(a, b, dn, preferred_element_type=f32)


def dot2(a, b, dn=NN):
    h = a.shape[0] // 2
    return jnp.concatenate([dot(a[:h], b, dn), dot(a[h:], b, dn)], axis=0)


def split_rows(x, g):
    r, c = x.shape
    y = x.reshape(r // (2 * g), 2 * g, c)
    return y[:, :g].reshape(r // 2, c), y[:, g:].reshape(r // 2, c)


def merge_rows(a, b, g):
    r, c = a.shape
    return jnp.concatenate([a.reshape(r // g, g, c), b.reshape(r // g, g, c)], axis=1).reshape(2 * r, c)


def split_cols(x):
    n = x.shape[1] // 128
    ev = [x[:, 128 * i:128 * (i + 1)] for i in range(0, n, 2)]
    od = [x[:, 128 * i:128 * (i + 1)] for i in range(1, n, 2)]
    cat = lambda l: l[0] if len(l) == 1 else jnp.concatenate(l, axis=1)
    return cat(ev), cat(od)


def merge_cols(a, b):
    parts = []
    for i in range(a.shape[1] // 128):
        parts += [a[:, 128 * i:128 * (i + 1)], b[:, 128 * i:128 * (i + 1)]]
    return jnp.concatenate(parts, axis=1)


def pk(x):
    return pltpu.bitcast(x, u32)


def upk(x):
    return pltpu.bitcast(x, bf16)


def mem(j, n, r0=0, size=None):
    return slice(j * n + r0, j * n + r0 + (n if size is None else size))


def cat0(*xs):
    return jnp.concatenate(xs, axis=0)


def cat1(*xs):
    return jnp.concatenate(xs, axis=1)


def _block(per, mo, mv, in_buf, out_buf, dma, nsteps, staged, step, carry):
    fetch, fetch_wait, put, put_wait = dma
    scale = D ** -0.5
    c = scale * math.log2(math.e)
    plan_tab = PLAN_LOOP if staged is None else PLAN_FIRST
    arrived = set()
    mo = list(mo)
    mv = list(mv)
    cur = lax.bitwise_and(step, 1)

    def load(name, h, r0=0, r1=None, c0=0, c1=D):
        grp = 2 * h + (0 if name in ("q", "k") else 1)
        if staged is not None and grp not in arrived:
            arrived.add(grp)
            for cp in staged(grp):
                cp.wait()
        base = OFF[name] + h * ROWS[name]
        r1 = ROWS[name] if r1 is None else r1
        return in_buf[cur, base + r0:base + r1, c0:c1]

    def flip(l):
        l.reverse()
        return l[0]

    z0 = lax.shift_right_logical(step, 20)
    z1 = lax.shift_right_logical(step, 21)
    z2 = lax.shift_right_logical(step, 22)
    never = lax.broadcasted_iota(jnp.int32, (8, 128), 0) < z0
    st = [dict() for _ in range(HB)]
    delayed = []
    res = {}
    todo = {}

    def emit(name, h, val, delay):
        r0 = OFF[name] + h * ROWS[name]
        out_buf[cur, r0:r0 + ROWS[name]] = val
        put(name, h, step, cur, cur + z1)
        token(pk(out_buf[cur + z2, r0:r0 + 16, 0:128]), delay)

    masks = {n: never if n == 1 else jnp.concatenate([never] * n, axis=1) for n in (1, 2, 3, 4)}
    nv = masks.get

    def token(tok, delay):
        delayed.append([tok, delay])

    def deadline(x, delay):
        for t in range(x.shape[1] // 128):
            token(pk(jnp.broadcast_to(x[:, 128 * t:128 * (t + 1)], (8, 128))), delay)

    def tie(x):
        now = [e[0] for e in delayed if e[1] <= 0]
        delayed[:] = [[e[0], e[1] - 1] for e in delayed if e[1] > 0]
        if not now:
            return x
        head = lax.select(never, functools.reduce(lambda a, b: a | b, now), pk(x[0:16, 0:128]))
        top = upk(head) if x.shape[1] == 128 else cat1(upk(head), x[0:16, 128:])
        return cat0(top, x[16:])

    def gate(x, trig, n=None):
        w = x.shape[1] // 128
        n = w if n is None else min(n, w)
        g = lax.select(nv(n), trig if n == 1 else jnp.concatenate([trig] * n, axis=1), x if n == w else x[:, :128 * n])
        return g if n == w else cat1(g, x[:, 128 * n:])

    def gate_top(x, trig):
        return cat0(gate(x[0:8], trig), x[8:16])

    def trig_of(name, frac):
        m = res[name]
        if name[0] in "OQ":
            k = min(int(frac * 32), 31)
            return m[8 * (k % 16):8 * (k % 16) + 8, 128 * (k // 16):128 * (k // 16) + 128]
        rows = m.shape[0] // 2 if name[0] in "VKP" else m.shape[0]
        k = min(int(frac * (rows // 8)), rows // 8 - 1)
        return m[8 * k:8 * k + 8, 0:128]

    def slot(name, lhs, rhs, d):
        for f in todo.pop(SLOT_INDEX[name], []):
            f()
        m = d(lhs(), tie(rhs()))
        res[name] = m
        return m

    def plan(key, unit, after=None, final=None, off=None):
        items = plan_tab[key]
        base = 0
        for n, (name, cnt) in enumerate(items):
            def run(name=name, cnt=cnt, base=base, last=(n == len(items) - 1)):
                for k in range(cnt):
                    unit(base + k, lambda x=0.0, k=k: trig_of(name, (k + x) / cnt))
                if after is not None:
                    after()
                if last and final is not None:
                    final()
            at = SLOT_INDEX[name] + (off if off is not None else (1 if name[0] == "S" else 2))
            todo.setdefault(at, []).append(run)
            base += cnt

    def strassen(g, A, B, scr, d):
        ms = []
        for n, (ja, jb) in enumerate([(2, 2), (1, 5), (4, 1), (3, 0), (0, 6), (6, 3), (5, 4)]):
            m = slot(f"{g}{n}", lambda: A(ja), lambda: B(jb), d)
            ms.append(m)
            if n < 5:
                scr[z0, mem(n, m.shape[0])] = m
        L = lambda n: scr[z2, mem(n, ms[0].shape[0])]
        m7, m6 = ms[5], ms[6]
        return (L(0) + L(1) - L(2) + m7, L(4) + L(2), L(3) + L(1), L(0) - L(3) + L(4) + m6)

    def vk_unit(h, name, ch, tf):
        src, sc = ("v", per[h]["vt"]) if name == "VT" else ("k", per[h]["kt"])
        us = [[] for _ in range(5)]
        for g in range(8):
            r0 = 256 * ch + 32 * g
            x = load(src, h, r0, r0 + 32).astype(f32)
            tr = tf(g / 8 * 1.0)
            a = gate_top(x[:16, :128], tr); b = x[:16, 128:]; cc = x[16:, :128]; d = gate_top(x[16:, 128:], tr)
            for l, u in zip(us, [a + d, b + d, a + cc, b - a, cc - d]):
                l.append(u)
            if name == "VT":
                r = 128 * ch + 16 * g
                wz = (z0, z1)[g % 2]
                per[h]["vn"][wz, mem(0, 512, r, 16)] = cat1(us[0][-1], us[1][-1]).astype(bf16)
                per[h]["vn"][wz, mem(1, 512, r, 16)] = cat1(us[2][-1], us[3][-1]).astype(bf16)
                if g % 2 == 1:
                    r5 = 64 * ch + 16 * (g // 2)
                    per[h]["vn5"][z0, r5:r5 + 16, :] = cat1(us[4][-2], us[4][-1]).astype(bf16)
        top, bot = split_rows(load(src, h, 256 * ch, 256 * (ch + 1)), GK)
        x11, _ = split_cols(top)
        _, x22 = split_cols(bot)
        for j, y in enumerate([x11, x22] + [cat0(*l).astype(bf16) for l in us]):
            sc[z0, mem(j, 64), 128 * ch:128 * (ch + 1)] = pk(y.T)

    def vk_token(h, name):
        sc = per[h]["vt"] if name == "VT" else per[h]["kt"]
        token(sc[z2, 0:8, 0:128], 2)
        if name == "VT":
            token(pk(per[h]["vn"][z2, 0:16, 0:128]) | pk(per[h]["vn5"][z2, 0:16, 0:128]), 2)

    def w_unit(h, which, g, tf):
        src = ("do", "q")[which]
        r0 = 256 * (g // 4) + 32 * (g % 4)
        t5 = []
        for e in range(2):
            tr = tf(e / 2)
            x = load(src, h, r0 + 16 * e, r0 + 16 * e + 16).astype(f32)
            y = load(src, h, r0 + 128 + 16 * e, r0 + 144 + 16 * e).astype(f32)
            a = gate_top(x[:, :128], tr); b = x[:, 128:]; cc = y[:, :128]; d = gate_top(y[:, 128:], tr)
            r = 32 * g + 16 * e
            wz = (z0, z1)[e]
            per[h]["w"][wz, mem(2 * which, 256, r, 16)] = cat1(a + d, cc + d).astype(bf16)
            per[h]["w"][wz, mem(2 * which + 1, 256, r, 16)] = cat1(a + b, cc - a).astype(bf16)
            t5.append(b - d)
        per[h]["w5"][z0, mem(which, 128, 16 * g, 16)] = cat1(*t5).astype(bf16)

    def w_token(h, which):
        token(pk(per[h]["w"][z2, mem(2 * which, 256, 0, 16), 0:128])
              | pk(per[h]["w5"][z2, mem(which, 128, 0, 16), 0:128]), 2)

    def get_w(h, which):
        src = ("do", "q")[which]

        def f(j):
            if j == 0:
                return cat0(load(src, h, 0, 128, 0, 128), load(src, h, 256, 384, 0, 128))
            if j == 1:
                return cat0(load(src, h, 128, 256, 128, 256), load(src, h, 384, 512, 128, 256))
            if j < 6:
                return per[h]["w"][z2, mem(2 * which + (j - 2) // 2, 256), 128 * (j % 2):128 * (j % 2 + 1)]
            return merge_rows(per[h]["w5"][z0, mem(which, 128), 0:128],
                              per[h]["w5"][z0, mem(which, 128), 128:256], 16)
        return f

    def get_vn(h, j):
        if j < 2:
            t, bt = split_rows(load("v", h), GK)
            return t[:, 0:128] if j == 0 else bt[:, 128:256]
        if j < 6:
            return per[h]["vn"][z2, mem((j - 2) // 2, 512), 128 * (j % 2):128 * (j % 2 + 1)]
        return merge_rows(per[h]["vn5"][z0, :, 0:128], per[h]["vn5"][z0, :, 128:256], 16)

    get_p = lambda h: (lambda j: per[h]["p"][z2, mem(j, 512)])
    get_ds = lambda h: (lambda j: per[h]["ds"][z2, mem(j, 512)])
    get_t = lambda h, name: (lambda j: upk(per[h][name][z0, mem(j, 64)]))

    def grp_s(h):
        R = 8 * FLY
        st[h]["m"] = []
        for t in range(2):
            acc = None
            for u in range(2):
                s = slot(f"S{'ab'[h]}{2 * t + u}", lambda: load("k", h, SUB * u, SUB * (u + 1)),
                         lambda: load("q", h, 256 * t, 256 * (t + 1)), lambda a, b: dot(a, b, NT) * c)
                for g in range(SUB // R):
                    x = s[R * g:R * (g + 1)]
                    mx = jnp.max(x.reshape(FLY, 8, 256), axis=0)
                    acc = mx if acc is None else jnp.maximum(acc, mx)
                    x = cat0(x[:R - 8], lax.select(nv(2), acc, x[R - 8:]))
                    per[h]["s"][z0, SUB * u + R * g:SUB * u + R * (g + 1), 256 * t:256 * (t + 1)] = x
            m = jnp.max(acc, axis=0, keepdims=True)
            st[h]["m"].append(m)
            st[h][f"m8{t}"] = jnp.broadcast_to(m, (8, 256))
            deadline(m, 1)

    def sum_unit(h, t, g, tf):
        mg = gate(st[h][f"m8{t}"], tf(), 2)
        e = jnp.exp2(per[h]["s"][z0, R1 * g:R1 * (g + 1), 256 * t:256 * (t + 1)].reshape(R1 // 8, 8, 256)
                     - mg[None]).reshape(R1, 256)
        while e.shape[0] > 8:
            e = e[:e.shape[0] // 2] + e[e.shape[0] // 2:]
        st[h][f"acc{t}"] = e if g == 0 else st[h][f"acc{t}"] + e

    def join4(x):
        comb = x[:, 0:128] + x[:, 128:256] + x[:, 256:384] + x[:, 384:512]
        return lax.select(nv(4)[0:1], jnp.concatenate([comb] * 4, axis=1), x)

    def sum_final(h, t):
        l = jnp.sum(st[h][f"acc{t}"], axis=0, keepdims=True)
        st[h][f"bb{t}"] = st[h]["m"][t] + jnp.log2(l)
        if "bb0" in st[h] and "bb1" in st[h]:
            bb = join4(cat1(st[h]["bb0"], st[h]["bb1"]))
            st[h]["b8"] = jnp.broadcast_to(bb, (8, 512))
            deadline(bb, 0 + (1 if plan_tab["p1" + "ab"[h] + "1"][-1][0][0] == "S" else 0))

    def prob_unit(h, g, tf):
        bg = gate(st[h]["b8"], tf(), 4)
        r0 = 32 * (g // 2) + 8 * (g % 2)
        a, b = split_cols(jnp.exp2(per[h]["s"][z0, r0:r0 + 8, :] - bg))
        cc, d = split_cols(jnp.exp2(per[h]["s"][z0, r0 + 16:r0 + 24, :] - bg))
        wz = (z0, z1)[g % 2]
        for j, x in enumerate([a, d, a + d, cc + d, a + b, cc - a, b - d, b, cc]):
            per[h]["p"][wz, mem(j, 512, 8 * g, 8)] = x.astype(bf16)

    def grp_o(h):
        c11, c12, c21, c22 = strassen("O" + "ab"[h], get_t(h, "vt"), get_p(h), flip(mo), dot)
        top = merge_cols(c11, c12); bot = merge_cols(c21, c22)
        emit("o", h, cat1(top.T, bot.T).astype(bf16), 4)

    def grp_v(h):
        c11, c12, c21, c22 = strassen("V" + "ab"[h], get_p(h), get_w(h, 0), flip(mv), dot2)
        emit("dv", h, merge_rows(cat1(c11, c12), cat1(c21, c22), GK).astype(bf16), 2)

    def grp_p(h):
        W = get_w(h, 0)
        for n, (ja, jb) in enumerate([(2, 2), (1, 4), (5, 1), (3, 6), (6, 0), (0, 3), (4, 5)]):
            per[h]["mp"][z0, mem(n, 512)] = slot(f"P{'ab'[h]}{n}", lambda: get_vn(h, ja), lambda: W(jb),
                                                 lambda a, b: dot2(a, b, NT))

    def pdp_unit(h, g, tf):
        rs = slice(8 * g, 8 * (g + 1))
        M = lambda n: per[h]["mp"][z2, mem(n, 512, 8 * g, 8)]
        m1 = gate(M(0), tf(), 2); n4 = M(1); n5 = M(2); n2 = M(4); n3 = M(5)
        pp = lambda j: per[h]["p"][z2, mem(j, 512, 8 * g, 8)].astype(f32)
        t11 = ((m1 + M(3)) - n4 + n5) * pp(0)
        t12 = (n3 + n5) * pp(7)
        t21 = (n2 + n4) * pp(8)
        t22 = ((m1 + M(6)) - n3 + n2) * pp(1)
        wz = (z0, z1)[g % 2]
        per[h]["s"][wz, rs, :] = cat1(t11, t12)
        per[h]["s"][wz, 512 + 8 * g:512 + 8 * (g + 1), :] = cat1(t21, t22)
        e = cat1(t11 + t21, t12 + t22)
        st[h]["dacc"] = e if g == 0 else st[h]["dacc"] + e

    def pdp_final(h):
        delta = join4(jnp.sum(st[h]["dacc"], axis=0, keepdims=True))
        st[h]["d8"] = jnp.broadcast_to(delta, (8, 512))
        deadline(delta, 1 + (1 if plan_tab["d1" + "ab"[h]][-1][0][0] == "S" else 0))

    def ds_unit(h, g, tf):
        d8 = gate(st[h]["d8"], tf(), 1)
        de, do_ = d8[:, 0:256], d8[:, 256:512]
        rs = slice(8 * g, 8 * (g + 1))
        top = per[h]["s"][z2, rs, :]; bot = per[h]["s"][z2, 512 + 8 * g:512 + 8 * (g + 1), :]
        pp = lambda j: per[h]["p"][z2, mem(j, 512, 8 * g, 8)].astype(f32)
        a = top[:, :256] - pp(0) * de; b = top[:, 256:] - pp(7) * do_
        cc = bot[:, :256] - pp(8) * de; d = bot[:, 256:] - pp(1) * do_
        wz = (z0, z1)[g % 2]
        for j, x in enumerate([a, d, a + d, cc + d, a + b, cc - a, b - d]):
            per[h]["ds"][wz, mem(j, 512, 8 * g, 8)] = x.astype(bf16)

    def grp_k(h):
        c11, c12, c21, c22 = strassen("K" + "ab"[h], get_ds(h), get_w(h, 1), flip(mv), dot2)
        emit("dk", h, (merge_rows(cat1(c11, c12), cat1(c21, c22), GK) * scale).astype(bf16), 2)

    def grp_q(h):
        c11, c12, c21, c22 = strassen("Q" + "ab"[h], get_t(h, "kt"), get_ds(h), flip(mo), dot)
        top = merge_cols(c11, c12) * scale; bot = merge_cols(c21, c22) * scale
        emit("dq", h, cat1(top.T, bot.T).astype(bf16), 4)

    P = functools.partial
    for h in range(HB):
        x = "ab"[h]
        plan("y" + x, P(vk_unit, h, "VT"), after=P(vk_token, h, "VT"), off=1)
        plan("z" + x, P(vk_unit, h, "KT"), after=P(vk_token, h, "KT"), off=1)
        plan("w" + x, P(w_unit, h, 0), after=P(w_token, h, 0), off=1)
        plan("u" + x, P(w_unit, h, 1), after=P(w_token, h, 1), off=1)
        plan("p1" + x + "0", P(sum_unit, h, 0), final=P(sum_final, h, 0))
        plan("p1" + x + "1", P(sum_unit, h, 1), final=P(sum_final, h, 1))
        plan("p2" + x, P(prob_unit, h), after=lambda h=h: token(pk(per[h]["p"][z2, 0:16, 0:128]), 1))
        plan("d1" + x, P(pdp_unit, h), after=lambda h=h: token(pk(per[h]["s"][z2, 0:8, 0:128]), 1),
             final=P(pdp_final, h))
        plan("ds" + x, P(ds_unit, h), after=lambda h=h: token(pk(per[h]["ds"][z2, 0:16, 0:128]), 1))
    groups = dict(S=grp_s, O=grp_o, V=grp_v, P=grp_p, K=grp_k, Q=grp_q)
    for g in ORDER:
        groups[g[0]]("ab".index(g[1]))
    assert not todo

    @pl.when(step + 2 < nsteps)
    def _():
        fetch(step + 2, cur)

    @pl.when(step + 1 < nsteps)
    def _():
        fetch_wait(1 - cur)

    if staged is None:
        put_wait(1 - cur)
    return carry


def _kernel(nsteps, q_hbm, k_hbm, v_hbm, do_hbm, o_hbm, dq_hbm, dk_hbm, dv_hbm, *scr):
    n = len(PER_HEAD)
    per = [dict(zip(PER_HEAD, scr[n * h:n * (h + 1)])) for h in range(HB)]
    mo = list(scr[n * HB:n * HB + 2])
    mv = list(scr[n * HB + 2:n * HB + 4])
    in_buf, out_buf, in_sem, out_sem, aux_sem = scr[n * HB + 4:n * HB + 9]
    hbm = dict(q=q_hbm, k=k_hbm, v=v_hbm, do=do_hbm, o=o_hbm, dq=dq_hbm, dk=dk_hbm, dv=dv_hbm)

    def fetch(it, sl):
        for name in INS:
            r = HB * ROWS[name]
            pltpu.make_async_copy(hbm[name].at[pl.ds(it * r, r)], in_buf.at[sl, pl.ds(OFF[name], r)],
                                  in_sem.at[sl]).start()

    def fetch_wait(sl):
        pltpu.make_async_copy(in_buf.at[sl], in_buf.at[sl], in_sem.at[sl]).wait()

    def put(name, h, it, sl, src_sl):
        r = ROWS[name]
        pltpu.make_async_copy(out_buf.at[src_sl, pl.ds(OFF[name] + h * r, r)],
                              hbm[name].at[pl.ds((it * HB + h) * r, r)], out_sem.at[sl]).start()

    def put_wait(sl):
        pltpu.make_async_copy(out_buf.at[sl], out_buf.at[sl], out_sem.at[sl]).wait()

    def staged(grp):
        h, names = grp // 2, (("q", "k"), ("v", "do"))[grp % 2]
        return [pltpu.make_async_copy(hbm[name].at[pl.ds(h * ROWS[name], ROWS[name])],
                                      in_buf.at[0, pl.ds(OFF[name] + h * ROWS[name], ROWS[name])],
                                      aux_sem.at[grp]) for name in names]

    pid = pl.program_id(0)
    args = (per, mo, mv, in_buf, out_buf, (fetch, fetch_wait, put, put_wait), nsteps)

    @pl.when(pid == 0)
    def _():
        for grp in range(2 * HB):
            for cp in staged(grp):
                cp.start()
        fetch(1, 1)
        _block(*args, staged, pid, 0)

    @pl.when(pid == 1)
    def _():
        lax.fori_loop(1, nsteps, functools.partial(_block, *args, None), 0)
        put_wait((nsteps - 1) % 2)


@jax.jit
def pallas_standalone__mha_softmax__near_ridge_kernel(q: jax.Array, k: jax.Array, v: jax.Array,
                                                      grad_out: jax.Array):
    B, H = q.shape[:2]
    assert q.shape[2:] == (SQ, D) and k.shape[2:] == (SK, D) and (B * H) % HB == 0 and B * H >= 2 * HB
    q2, k2, v2, do2 = (x.reshape(-1, D) for x in (q, k, v, grad_out))
    vm = pltpu.VMEM
    per = [vm((1, SK, SQ), f32), vm((1, 9 * 512, 256), bf16), vm((1, 7 * 512, 256), bf16),
           vm((1, 7 * 64, 512), u32), vm((1, 7 * 64, 512), u32), vm((1, 7 * 512, 256), f32),
           vm((1, 2 * 512, 256), bf16), vm((1, 256, 256), bf16), vm((1, 4 * 256, 256), bf16),
           vm((1, 2 * 128, 256), bf16)]
    shared = [vm((1, 5 * 128, 256), f32), vm((1, 5 * 128, 256), f32), vm((1, 5 * 512, 128), f32),
              vm((1, 5 * 512, 128), f32), vm((2, TOT, D), bf16), vm((2, TOT, D), bf16),
              pltpu.SemaphoreType.DMA((2,)), pltpu.SemaphoreType.DMA((2,)), pltpu.SemaphoreType.DMA((2 * HB,))]
    o, dq, dk, dv = pl.pallas_call(
        functools.partial(_kernel, B * H // HB),
        grid=(2,),
        in_specs=[pl.BlockSpec(memory_space=pl.ANY)] * 4,
        out_specs=[pl.BlockSpec(memory_space=pl.ANY)] * 4,
        out_shape=[jax.ShapeDtypeStruct(q2.shape, bf16), jax.ShapeDtypeStruct(q2.shape, bf16),
                   jax.ShapeDtypeStruct(k2.shape, bf16), jax.ShapeDtypeStruct(k2.shape, bf16)],
        scratch_shapes=per * HB + shared,
        compiler_params=pltpu.CompilerParams(dimension_semantics=("arbitrary",),
                                             vmem_limit_bytes=100 * 1024 * 1024,
                                             disable_bounds_checks=True),
    )(q2, k2, v2, do2)
    return o.reshape(q.shape), dq.reshape(q.shape), dk.reshape(k.shape), dv.reshape(k.shape)
```
